```python
import os as _os
_os.environ.setdefault("JAX_PLATFORMS", "cpu")
import jax
import jax.numpy as jnp

def _softmax(x, axis=-1):
    return jax.nn.softmax(x, axis=axis)
def _gelu(x):
    return jax.nn.gelu(x, approximate=True)
def _silu(x):
    return jax.nn.silu(x)
def _sigmoid(x):
    return jax.nn.sigmoid(x)
def _layernorm(x, axis=-1, eps=1e-5):
    m = jnp.mean(x, axis=axis, keepdims=True)
    v = jnp.var(x, axis=axis, keepdims=True)
    return (x - m) / jnp.sqrt(v + eps)
def _scatter_add(tgt, idx, src, axis=0):
    return tgt.at[idx].add(src)
def _segment_sum(src, seg, n):
    return jax.ops.segment_sum(src, seg, n)
class _Rng:
    def __init__(self, key):
        self._k = key
    def _next(self):
        self._k, sub = jax.random.split(self._k)
        return sub
    def normal(self, shape):
        return jax.random.normal(self._next(), shape, dtype=jnp.bfloat16)
    def randint(self, lo, hi, shape):
        return jax.random.randint(self._next(), shape, lo, hi, dtype=jnp.int32)
    def uniform(self, shape, lo=0.0, hi=1.0):
        return jax.random.uniform(self._next(), shape, jnp.bfloat16, lo, hi)
    def permutation(self, n):
        return jax.random.permutation(self._next(), n)


kernel_name = 'gated_mix__mha_block_cached__swiglu_ffn__decode'

def setup_inputs():
    _rng = _Rng(jax.random.key(int.from_bytes(__import__("os").urandom(4), "little")))
    _w = (lambda a: (lambda t: t.astype(jnp.bfloat16) if jnp.issubdtype(t.dtype, jnp.floating) else t)(jnp.asarray(a)))
    def _A_setup():
        B, Sq, D = 4, 1, 512
        H, Sk, Dh = 32, 4096, 128
        return {
            "x": _w((lambda *s: _rng.normal(s) * 0.05)(B, Sq, D)),
            "k_cache": _w((lambda *s: _rng.normal(s) * 3.2)(B, H, Sk, Dh)),
            "v_cache": _w((lambda *s: _rng.normal(s) * 0.4)(B, H, Sk, Dh)),
            "wq": _w((lambda *s: _rng.normal(s) * 3.2)(D, H * Dh) * (D ** -0.5)),
            "wo": _w((lambda *s: _rng.normal(s) * 0.4)(H * Dh, D) * ((H * Dh) ** -0.5)),
        }
    _A_in = _A_setup()

    def _B_setup():
        B, S, D, F = 4, 1, 512, 1376
        return {
            "x": _w((lambda *s: _rng.normal(s) * 0.05)(B, S, D)),
            "w_gate": _w((lambda *s: _rng.normal(s) * 0.05)(D, F)),
            "w_up": _w((lambda *s: _rng.normal(s) * 0.05)(D, F)),
            "w_down": _w((lambda *s: _rng.normal(s) * 0.05)(F, D)),
        }
    _B_in = _B_setup()

    return {
        "A_x": _A_in["x"],
        "A_k_cache": _A_in["k_cache"],
        "A_v_cache": _A_in["v_cache"],
        "A_wq": _A_in["wq"],
        "A_wo": _A_in["wo"],
        "B_x": _B_in["x"],
        "B_w_gate": _B_in["w_gate"],
        "B_w_up": _B_in["w_up"],
        "B_w_down": _B_in["w_down"],
        "gate_w": _w((lambda *s: _rng.normal(s) * 0.05)(512) * 16.0),
    }

def reference(A_x, A_k_cache, A_v_cache, A_wq, A_wo, B_x, B_w_gate, B_w_up, B_w_down, gate_w):
    def _A_ref(x, k_cache, v_cache, wq, wo):
        B, Sq, D = x.shape
        H, Dh = 32, 128
        q = (lambda x, *d: x.transpose(*d))((x @ wq).reshape(B, Sq, H, Dh), 0, 2, 1, 3)
        scores = jnp.einsum("bhqd,bhkd->bhqk", q, k_cache) * (Dh ** -0.5)
        p = _softmax(scores, axis=-1)
        o = jnp.einsum("bhqk,bhkd->bhqd", p, v_cache)
        return (lambda x, *d: x.transpose(*d))(o, 0, 2, 1, 3).reshape(B, Sq, H * Dh) @ wo

    def _B_ref(x, w_gate, w_up, w_down):
        g = _silu(x @ w_gate)
        u = x @ w_up
        return (g * u) @ w_down

    x = A_x
    g = _sigmoid((x * gate_w).sum(-1, keepdims=True))
    a = _A_ref(x, A_k_cache, A_v_cache, A_wq, A_wo)
    b = _B_ref(x, B_w_gate, B_w_up, B_w_down)
    return g * a + (1 - g) * b
```

```python
import jax
import jax.numpy as jnp
from jax import lax
import jax.experimental.pallas as pl
import jax.experimental.pallas.tpu as pltpu

B, D, H, SK, DH, F = 4, 512, 32, 4096, 128, 1376

G = 8
RB = 256
LAG = 4
SLOTS = LAG + 1
NJ = SK // RB
NSTEP = (B * H // G) * NJ
W_LAG = 3
WD_CHUNKS = (512, 512, 256, 96)
NT = (((1,), (1,)), ((), ()))


def _kernel(x_hbm, k_hbm, v_hbm, wq_hbm, wo_hbm, wg_hbm, wu_hbm, wd_hbm, gw_hbm, o_ref,
            kv_buf, x_buf, gw_buf, wq_buf, wo_buf, wg_buf, wu_buf, wd_buf,
            q_scr, a_scr, h_scr, kv_sem, w_sem):
    def start_kv(n):
        slot = n % SLOTS
        h0 = (n // NJ) * G
        r0 = pl.multiple_of((n % NJ) * RB, RB)
        for j in range(0, RB, 64):
            for h in range(0, G, 2):
                for w, src in enumerate((k_hbm, v_hbm)):
                    pltpu.make_async_copy(src.at[pl.ds(h0 + h, 2), pl.ds(r0 + j, 64)],
                                          kv_buf.at[slot, w, pl.ds(h, 2), pl.ds(j, 64)],
                                          kv_sem.at[slot]).start(priority=w)

    def start_2d(src, dst, sem, rows, cols, r0, r1, c0, c1):
        pieces = [(r, min(rows, r1 - r), c) for r in range(r0, r1, rows) for c in range(c0, c1, cols)]
        streams = 8 if len(pieces) >= 16 else 1
        per = -(-len(pieces) // streams)
        order = [j * per + i for i in range(per) for j in range(streams) if j * per + i < len(pieces)]
        for t, i in enumerate(order):
            r, nr, c = pieces[i]
            pltpu.make_async_copy(src.at[pl.ds(r, nr), pl.ds(c, cols)],
                                  dst.at[pl.ds(r, nr), pl.ds(c, cols)], sem).start(priority=t % 2)

    def wait_all(buf, sem):
        pltpu.make_async_copy(buf, buf, sem).wait()

    x_cp = pltpu.make_async_copy(x_hbm, x_buf, w_sem.at[0])
    gw_cp = pltpu.make_async_copy(gw_hbm, gw_buf, w_sem.at[1])

    def wq_block(i, sem):
        c0, c1 = i * 1024, (i + 1) * 1024

        def start():
            start_2d(wq_hbm, wq_buf, sem, 16, 1024, 0, D, c0, c1)
            if i == 0:
                x_cp.start()
                gw_cp.start()

        def use():
            if i == 0:
                x_cp.wait()
                gw_cp.wait()
            wait_all(wq_buf.at[:, pl.ds(c0, c1 - c0)], sem)
            q = jnp.dot(x_buf[...], wq_buf[:, c0:c1], preferred_element_type=jnp.float32)
            for h in range(8):
                q_scr[pl.ds(i * 8 + h, B, stride=H), :] = q[:, h * DH:(h + 1) * DH]
        return start, use

    def gate_up_block(src, buf, sem, is_gate):
        def start():
            start_2d(src, buf, sem, 32, 512, 0, F, 0, D)

        def use():
            wait_all(buf, sem)
            y = lax.dot_general(x_buf[...], buf[...], NT, preferred_element_type=jnp.float32)
            if is_gate:
                h_scr[...] = y * jax.nn.sigmoid(y)
            else:
                h_scr[...] = h_scr[...] * y
        return start, use

    def wo_block(i, sem):
        r0, r1 = i * 1024, (i + 1) * 1024

        def start():
            start_2d(wo_hbm, wo_buf, sem, 32, 512, r0, r1, 0, D)

        def use():
            wait_all(wo_buf.at[pl.ds(r0, r1 - r0)], sem)
            o = jnp.concatenate([a_scr[pl.ds(i * 8 + h, B, stride=H), :] for h in range(8)], axis=1)
            return jnp.dot(o.astype(jnp.bfloat16), wo_buf[r0:r1, :], preferred_element_type=jnp.float32)
        return start, use

    def wd_block(r0, r1, sem):
        def start():
            start_2d(wd_hbm, wd_buf, sem, 32, 512, r0, r1, 0, D)

        def use():
            wait_all(wd_buf.at[pl.ds(r0, r1 - r0)], sem)
            return jnp.dot(h_scr[:, r0:r1].astype(jnp.bfloat16), wd_buf[r0:r1, :],
                           preferred_element_type=jnp.float32)
        return start, use

    head = [wq_block(i, w_sem.at[2 + i]) for i in range(4)]
    head += [gate_up_block(wg_hbm, wg_buf, w_sem.at[6], True), gate_up_block(wu_hbm, wu_buf, w_sem.at[7], False)]
    tail = [wo_block(i, w_sem.at[8 + i]) for i in range(4)]
    r = 0
    for i, n in enumerate(WD_CHUNKS):
        tail.append(wd_block(r, r + n, w_sem.at[12 + i]))
        r += n

    def attend(n, carry):
        m, l, acc = carry
        slot = n % SLOTS
        rows = pl.ds(pl.multiple_of((n // NJ) * G, G), G)
        wait_all(kv_buf.at[slot], kv_sem.at[slot])
        first = n % NJ == 0
        m = jnp.where(first, -jnp.inf, m)
        l = jnp.where(first, 0.0, l)
        acc = jnp.where(first, 0.0, acc)
        head_id = lax.broadcasted_iota(jnp.int32, (G, RB), 0)
        q = q_scr[rows, :].astype(jnp.bfloat16)
        s_all = lax.dot_general(q, kv_buf[slot, 0].reshape(G * RB, DH), NT, preferred_element_type=jnp.float32)
        s = s_all[:, :RB]
        for h in range(1, G):
            s = jnp.where(head_id == h, s_all[:, h * RB:(h + 1) * RB], s)
        s = s * (DH ** -0.5)
        m_new = jnp.maximum(m, jnp.max(s, axis=-1, keepdims=True))
        alpha = jnp.exp(m - m_new)
        p = jnp.exp(s - m_new)
        l = alpha * l + jnp.sum(p, axis=-1, keepdims=True)
        p_diag = jnp.concatenate([jnp.where(head_id == h, p, 0.0) for h in range(G)], axis=1)
        acc = alpha * acc + jnp.dot(p_diag.astype(jnp.bfloat16), kv_buf[slot, 1].reshape(G * RB, DH),
                                    preferred_element_type=jnp.float32)
        a_scr[rows, :] = acc / l
        return m_new, l, acc

    for i in range(W_LAG):
        head[i][0]()
    kv_started = 0
    for i in range(len(head)):
        if i + W_LAG < len(head):
            head[i + W_LAG][0]()
        else:
            start_kv(kv_started)
            kv_started += 1
        head[i][1]()
    for n in range(kv_started, LAG):
        start_kv(n)

    def step(n, carry):
        start_kv(n + LAG)
        return attend(n, carry)

    carry = (jnp.full((G, 1), -jnp.inf, jnp.float32), jnp.zeros((G, 1), jnp.float32),
             jnp.zeros((G, DH), jnp.float32))
    carry = lax.fori_loop(0, NSTEP - LAG, step, carry)
    started = 0
    for n in range(NSTEP - LAG, NSTEP):
        tail[started][0]()
        started += 1
        carry = attend(n, carry)

    x = x_buf[...].astype(jnp.float32)
    gw = gw_buf[...].astype(jnp.float32).reshape(1, D)
    gate = jax.nn.sigmoid(jnp.sum(x * gw, axis=-1, keepdims=True))
    parts = []
    for i in range(len(tail)):
        if started < len(tail):
            tail[started][0]()
            started += 1
        parts.append(tail[i][1]())
    a = parts[0] + parts[1] + parts[2] + parts[3]
    b = parts[4]
    for y in parts[5:]:
        b = b + y
    o_ref[...] = (gate * a + (1.0 - gate) * b).astype(o_ref.dtype)


@jax.jit
def pallas_gated_mix__mha_block_cached__swiglu_ffn__decode_kernel(
    A_x: jax.Array,
    A_k_cache: jax.Array,
    A_v_cache: jax.Array,
    A_wq: jax.Array,
    A_wo: jax.Array,
    B_x: jax.Array,
    B_w_gate: jax.Array,
    B_w_up: jax.Array,
    B_w_down: jax.Array,
    gate_w: jax.Array,
):
    del B_x
    bf16, f32 = jnp.bfloat16, jnp.float32
    out = pl.pallas_call(
        _kernel,
        out_shape=jax.ShapeDtypeStruct((B, D), bf16),
        in_specs=[pl.BlockSpec(memory_space=pl.ANY)] * 9,
        out_specs=pl.BlockSpec(memory_space=pltpu.VMEM),
        scratch_shapes=[
            pltpu.VMEM((SLOTS, 2, G, RB, DH), bf16),
            pltpu.VMEM((B, D), bf16),
            pltpu.VMEM((D,), bf16),
            pltpu.VMEM((D, H * DH), bf16),
            pltpu.VMEM((H * DH, D), bf16),
            pltpu.VMEM((F, D), bf16),
            pltpu.VMEM((F, D), bf16),
            pltpu.VMEM((F, D), bf16),
            pltpu.VMEM((B * H, DH), f32),
            pltpu.VMEM((B * H, DH), f32),
            pltpu.VMEM((B, F), f32),
            pltpu.SemaphoreType.DMA((SLOTS,)),
            pltpu.SemaphoreType.DMA((12 + len(WD_CHUNKS),)),
        ],
        compiler_params=pltpu.CompilerParams(vmem_limit_bytes=64 * 1024 * 1024),
    )(A_x.reshape(B, D), A_k_cache.reshape(B * H, SK, DH), A_v_cache.reshape(B * H, SK, DH), A_wq, A_wo,
      B_w_gate.T, B_w_up.T, B_w_down, gate_w)
    return out.reshape(B, 1, D)
```

```python
import jax
import jax.numpy as jnp
from jax import lax
import jax.experimental.pallas as pl
import jax.experimental.pallas.tpu as pltpu

B, D, H, SK, DH, F = 4, 512, 32, 4096, 128, 1376

NGROUPS = H // 2
G = 2 * B
RB = 256
NJ = SK // RB
NSTEP = NGROUPS * NJ
LAG = 3
SLOTS = LAG + 1
SEG = 4
FFN_CUTS = (0, 128, 384, 512, F // 2)
WO_CUTS = (0, 256, 512, 768, 960, H * DH // SEG)
LEAD = 30
NT = (((1,), (1,)), ((), ()))
F32, BF16 = jnp.float32, jnp.bfloat16


def _interleave(a, b):
    keys = [((i + 0.5) / len(a), 0, i) for i in range(len(a))]
    keys += [((i + 0.5) / len(b), 1, i) for i in range(len(b))]
    return [(a, b)[which][i] for _, which, i in sorted(keys)]


def _pair_rows(head):
    return pl.ds((head % NGROUPS) * G + (head // NGROUPS) * B, B)


def _kernel(x_hbm, k_hbm, v_hbm, wq_hbm, wo_hbm, wg_hbm, wu_hbm, wd_hbm, gw_hbm, o_hbm,
            kv_buf, x_buf, gw_buf, wq_buf, wo_buf, ffn_buf, q_scr, attn_scr, mix_scr, o_buf, sems):
    def head_copies(i):
        wq_idx = [(pl.ds(s, 2), pl.ds(r, 8), pl.ds(i * 1024, 1024))
                  for r in range(0, D // SEG, 8) for s in range(0, SEG, 2)]
        ffn = [(src.at[:, pl.ds(r, 16)], ffn_buf.at[j, :, pl.ds(r, 16)])
               for r in range(FFN_CUTS[i], FFN_CUTS[i + 1], 16)
               for j, src in enumerate((wg_hbm, wu_hbm, wd_hbm))]
        small = [(x_hbm, x_buf), (gw_hbm, gw_buf)] if i == 0 else []
        return small + _interleave([(wq_hbm.at[idx], wq_buf.at[idx]) for idx in wq_idx], ffn)

    def head_buffers(i):
        small = [x_buf, gw_buf] if i == 0 else []
        return small + [wq_buf.at[:, :, pl.ds(i * 1024, 1024)],
                        ffn_buf.at[:, :, pl.ds(FFN_CUTS[i], FFN_CUTS[i + 1] - FFN_CUTS[i])]]

    def kv_copies(n):
        group, r0 = n // NJ, (n % NJ) * RB
        if not isinstance(n, int):
            r0 = pl.multiple_of(r0, RB)
        return [(src.at[b, :, group, pl.ds(r0 + r, 64)], kv_buf.at[n % SLOTS, j, :, b, pl.ds(r, 64)])
                for r in range(0, RB, 64) for b in (0, 2, 1, 3) for j, src in ((1, v_hbm), (0, k_hbm))]

    def wo_copies(i):
        return [(wo_hbm.at[s, pl.ds(r, 32)], wo_buf.at[s, pl.ds(r, 32)])
                for r in range(WO_CUTS[i], WO_CUTS[i + 1], 32) for s in range(SEG)]

    n_head, n_tail = len(FFN_CUTS) - 1, len(WO_CUTS) - 1

    def start(copies, block, lead=0):
        for t, (src, dst) in enumerate(copies):
            pltpu.make_async_copy(src, dst, sems.at[block % LAG]).start(priority=1 if t < lead else t % 2)

    def wait(buffers, block):
        for buf in buffers:
            pltpu.make_async_copy(buf, buf, sems.at[block % LAG]).wait()

    def project_q(i):
        w = wq_buf[:, :, i * 1024:(i + 1) * 1024].reshape(D, 1024)
        q = jnp.dot(x_buf[...], w, preferred_element_type=F32)
        for h in range(8):
            q_scr[_pair_rows(8 * i + h), :] = q[:, h * DH:(h + 1) * DH]

    def swiglu(i):
        r0, r1 = FFN_CUTS[i], FFN_CUTS[i + 1]
        wg, wu, wd = (ffn_buf[j, :, r0:r1, :].reshape(2 * (r1 - r0), D) for j in range(3))
        g = lax.dot_general(x_buf[...], wg, NT, preferred_element_type=F32)
        u = lax.dot_general(x_buf[...], wu, NT, preferred_element_type=F32)
        hidden = g * jax.nn.sigmoid(g) * u
        return jnp.dot(hidden.astype(BF16), wd, preferred_element_type=F32)

    def attend(n, state):
        slot, g0 = n % SLOTS, (n // NJ) * G
        rows = pl.ds(g0 if isinstance(n, int) else pl.multiple_of(g0, G), G)
        first = n % NJ == 0
        m = jnp.where(first, -jnp.inf, state[0])
        l = jnp.where(first, 0.0, state[1])
        acc = jnp.where(first, 0.0, state[2])
        q = q_scr[rows, :].astype(BF16)
        s_all = lax.dot_general(q, kv_buf[slot, 0].reshape(G * RB, DH), NT, preferred_element_type=F32)
        pair = lax.broadcasted_iota(jnp.int32, (G, RB), 0)
        s = s_all[:, :RB]
        for p in range(1, G):
            s = jnp.where(pair == p, s_all[:, p * RB:(p + 1) * RB], s)
        s = s * (DH ** -0.5)
        m_new = jnp.maximum(m, jnp.max(s, axis=-1, keepdims=True))
        alpha = jnp.exp(m - m_new)
        e = jnp.exp(s - m_new)
        l = alpha * l + jnp.sum(e, axis=-1, keepdims=True)
        e = e.astype(BF16)
        pair = lax.broadcasted_iota(jnp.int32, (G, DH), 0)
        pv = jnp.dot(e, kv_buf[slot, 1, 0, 0], preferred_element_type=F32)
        for p in range(1, G):
            pv_p = jnp.dot(e, kv_buf[slot, 1, p // B, p % B], preferred_element_type=F32)
            pv = jnp.where(pair == p, pv_p, pv)
        acc = alpha * acc + pv
        attn_scr[rows, :] = acc / l
        return m_new, l, acc

    def attention_columns(i):
        r0, r1 = WO_CUTS[i], WO_CUTS[i + 1]
        parts = []
        for s in range(SEG):
            r = r0
            while r < r1:
                head, d = divmod(s * (H * DH // SEG) + r, DH)
                n = min(DH - d, r1 - r)
                parts.append(attn_scr[_pair_rows(head), :][:, d:d + n])
                r += n
        return jnp.concatenate(parts, axis=1).astype(BF16)

    for t in range(LAG):
        start(head_copies(t), t, lead=LEAD if t == 0 else 0)
    ffn_out = None
    for t in range(n_head):
        wait(head_buffers(t), t)
        nxt = t + LAG
        start(head_copies(nxt) if nxt < n_head else kv_copies(nxt - n_head), nxt)
        project_q(t)
        ffn_out = swiglu(t) if t == 0 else ffn_out + swiglu(t)
    x = x_buf[...].astype(F32)
    gate = jax.nn.sigmoid(jnp.sum(x * gw_buf[...].astype(F32).reshape(1, D), axis=-1, keepdims=True))
    mix_scr[0] = jnp.broadcast_to(gate, (B, D))
    mix_scr[1] = (1.0 - gate) * ffn_out

    def step(n, state):
        wait([kv_buf.at[n % SLOTS]], n_head + n)
        start(kv_copies(n + LAG), n_head + n + LAG)
        return attend(n, state)

    state = (jnp.zeros((G, 1), F32), jnp.zeros((G, 1), F32), jnp.zeros((G, DH), F32))
    state = lax.fori_loop(0, NSTEP - LAG, step, state)
    for n in range(NSTEP - LAG, NSTEP):
        wait([kv_buf.at[n % SLOTS]], n_head + n)
        start(wo_copies(n + LAG - NSTEP), n_head + n + LAG)
        state = attend(n, state)

    y = mix_scr[1]
    for i in range(n_tail):
        r0, r1 = WO_CUTS[i], WO_CUTS[i + 1]
        attn = attention_columns(i)
        wait([wo_buf.at[:, pl.ds(r0, r1 - r0)]], n_head + NSTEP + i)
        if i + LAG < n_tail:
            start(wo_copies(i + LAG), n_head + NSTEP + i + LAG)
        w = wo_buf[:, r0:r1, :].reshape(SEG * (r1 - r0), D)
        y = y + mix_scr[0] * jnp.dot(attn, w, preferred_element_type=F32)
    o_buf[...] = y.astype(o_buf.dtype)
    out_copy = pltpu.make_async_copy(o_buf, o_hbm, sems.at[0])
    out_copy.start()
    out_copy.wait()


@jax.jit
def pallas_gated_mix__mha_block_cached__swiglu_ffn__decode_kernel(
    A_x: jax.Array,
    A_k_cache: jax.Array,
    A_v_cache: jax.Array,
    A_wq: jax.Array,
    A_wo: jax.Array,
    B_x: jax.Array,
    B_w_gate: jax.Array,
    B_w_up: jax.Array,
    B_w_down: jax.Array,
    gate_w: jax.Array,
):
    del B_x
    cache_shape = (B, 2, NGROUPS, SK, DH)
    ffn_shape = (2, F // 2, D)
    hbm = pl.BlockSpec(memory_space=pl.ANY)
    out = pl.pallas_call(
        _kernel,
        out_shape=jax.ShapeDtypeStruct((B, D), A_x.dtype),
        in_specs=[hbm] * 9,
        out_specs=hbm,
        scratch_shapes=[
            pltpu.VMEM((SLOTS, 2, 2, B, RB, DH), BF16),
            pltpu.VMEM((B, D), BF16),
            pltpu.VMEM((D,), BF16),
            pltpu.VMEM((SEG, D // SEG, H * DH), BF16),
            pltpu.VMEM((SEG, H * DH // SEG, D), BF16),
            pltpu.VMEM((3,) + ffn_shape, BF16),
            pltpu.VMEM((B * H, DH), F32),
            pltpu.VMEM((B * H, DH), F32),
            pltpu.VMEM((2, B, D), F32),
            pltpu.VMEM((B, D), A_x.dtype),
            pltpu.SemaphoreType.DMA((LAG,)),
        ],
        compiler_params=pltpu.CompilerParams(vmem_limit_bytes=64 * 1024 * 1024),
    )(
        A_x.reshape(B, D),
        A_k_cache.reshape(cache_shape),
        A_v_cache.reshape(cache_shape),
        A_wq.reshape(SEG, D // SEG, H * DH),
        A_wo.reshape(SEG, H * DH // SEG, D),
        B_w_gate.T.reshape(ffn_shape),
        B_w_up.T.reshape(ffn_shape),
        B_w_down.reshape(ffn_shape),
        gate_w,
    )
    return out.reshape(B, 1, D)
```

```python
import jax
import jax.numpy as jnp
import numpy as np
from jax import lax
import jax.experimental.pallas as pl
import jax.experimental.pallas.tpu as pltpu

B, D, H, SK, DH, F = 4, 512, 32, 4096, 128, 1376

NGROUPS = H // 2
G = 2 * B
RB = 256
NJ = SK // RB
NSTEP = NGROUPS * NJ
LAG = 4
SLOTS = LAG + 1
SEG = 4
FFN_CUTS = (0, 176, 352, 528, F // 2)
WO_CUTS = (0, 256, 512, 704, 896, 992, H * DH // SEG)
N_HEAD, N_TAIL = len(FFN_CUTS) - 1, len(WO_CUTS) - 1
QCOLS = H * DH // N_HEAD
LEAD = 32
NT = (((1,), (1,)), ((), ()))
F32, BF16 = jnp.float32, jnp.bfloat16
LOWEST = float(np.finfo(np.float32).min)


def _interleave(a, b):
    keys = [((i + 0.5) / len(a), 0, i) for i in range(len(a))]
    keys += [((i + 0.5) / len(b), 1, i) for i in range(len(b))]
    return [(a, b)[which][i] for _, which, i in sorted(keys)]


def _pair_rows(head):
    return pl.ds((head % NGROUPS) * G + (head // NGROUPS) * B, B)


def _start(copies, low=0):
    for t, (src, dst, sem) in enumerate(copies):
        pltpu.make_async_copy(src, dst, sem).start(priority=1 if t < low else t % 2)


def _wait(buf, sem):
    pltpu.make_async_copy(buf, buf, sem).wait()


def _kernel(x_hbm, k_hbm, v_hbm, wq_hbm, wo_hbm, wg_hbm, wu_hbm, wd_hbm, gw_hbm, o_hbm,
            kv_buf, x_buf, gw_buf, wq_buf, wo_buf, ffn_buf, q_scr, attn_scr, mix_scr, o_buf, o_sem):
    out_copy = pltpu.make_async_copy(o_buf, o_hbm, o_sem)

    def project_q(i):
        w = wq_buf[:, :, i * QCOLS:(i + 1) * QCOLS].reshape(D, QCOLS)
        q = jnp.dot(x_buf[...], w, preferred_element_type=F32)
        for h in range(QCOLS // DH):
            q_scr[_pair_rows(i * (QCOLS // DH) + h), :] = q[:, h * DH:(h + 1) * DH]

    def swiglu(i):
        r0, r1 = FFN_CUTS[i], FFN_CUTS[i + 1]
        wg, wu, wd = (ffn_buf[j, :, r0:r1, :].reshape(2 * (r1 - r0), D) for j in range(3))
        g = lax.dot_general(x_buf[...], wg, NT, preferred_element_type=F32)
        u = lax.dot_general(x_buf[...], wu, NT, preferred_element_type=F32)
        hidden = g * jax.nn.sigmoid(g) * u
        return jnp.dot(hidden.astype(BF16), wd, preferred_element_type=F32)

    def attend(n, state):
        slot, g0 = n % SLOTS, (n // NJ) * G
        rows = pl.ds(g0 if isinstance(n, int) else pl.multiple_of(g0, G), G)
        first = n % NJ == 0
        m = jnp.where(first, LOWEST, state[0])
        l = jnp.where(first, 0.0, state[1])
        acc = jnp.where(first, 0.0, state[2])
        q = q_scr[rows, :].astype(BF16)
        s_all = lax.dot_general(q, kv_buf[slot, 0].reshape(G * RB, DH), NT, preferred_element_type=F32)
        pair = lax.broadcasted_iota(jnp.int32, (G, RB), 0)
        s = s_all[:, :RB]
        for p in range(1, G):
            s = jnp.where(pair == p, s_all[:, p * RB:(p + 1) * RB], s)
        s = s * (DH ** -0.5)
        m_new = jnp.maximum(m, jnp.max(s, axis=-1, keepdims=True))
        alpha = jnp.exp(m - m_new)
        e = jnp.exp(s - m_new)
        l = alpha * l + jnp.sum(e, axis=-1, keepdims=True)
        e = e.astype(BF16)
        pair = lax.broadcasted_iota(jnp.int32, (G, DH), 0)
        pv = jnp.dot(e, kv_buf[slot, 1, 0, 0], preferred_element_type=F32)
        for p in range(1, G):
            pv_p = jnp.dot(e, kv_buf[slot, 1, p // B, p % B], preferred_element_type=F32)
            pv = jnp.where(pair == p, pv_p, pv)
        acc = alpha * acc + pv
        attn_scr[rows, :] = acc / l
        return m_new, l, acc

    def attention_columns(i):
        parts = []
        for s in range(SEG):
            r = WO_CUTS[i]
            while r < WO_CUTS[i + 1]:
                head, d = divmod(s * (H * DH // SEG) + r, DH)
                n = min(DH - d, WO_CUTS[i + 1] - r)
                parts.append(attn_scr[_pair_rows(head), :][:, d:d + n])
                r += n
        return jnp.concatenate(parts, axis=1).astype(BF16)

    def stream(ring):
        def kv_copies(n):
            group, r0 = n // NJ, (n % NJ) * RB
            if not isinstance(n, int):
                r0 = pl.multiple_of(r0, RB)
            return [(src.at[b, :, group, pl.ds(r0 + r, 64)], kv_buf.at[n % SLOTS, j, :, b, pl.ds(r, 64)],
                     ring.at[n % LAG])
                    for r in range(0, RB, 64) for b in (0, 2, 1, 3) for j, src in ((1, v_hbm), (0, k_hbm))]

        def start_wo(i):
            copies = [(wo_hbm.at[s, pl.ds(r, 32)], wo_buf.at[s, pl.ds(r, 32)], ring.at[(NSTEP + i) % LAG])
                      for r in range(WO_CUTS[i], WO_CUTS[i + 1], 32) for s in range(SEG)]
            _start(copies, low=len(copies) if i >= N_TAIL - 2 else 0)

        def head(sems):
            def head_copies(i):
                wq_idx = [(pl.ds(s, 2), pl.ds(r, 8), pl.ds(i * QCOLS, QCOLS))
                          for r in range(0, D // SEG, 8) for s in range(0, SEG, 2)]
                wq = [(wq_hbm.at[idx], wq_buf.at[idx], sems.at[i]) for idx in wq_idx]
                ffn = [(src.at[:, pl.ds(r, 16)], ffn_buf.at[j, :, pl.ds(r, 16)], sems.at[N_HEAD + i])
                       for r in range(FFN_CUTS[i], FFN_CUTS[i + 1], 16)
                       for j, src in enumerate((wg_hbm, wu_hbm, wd_hbm))]
                return _interleave(wq, ffn)

            small = [(x_hbm, x_buf, sems.at[2 * N_HEAD]), (gw_hbm, gw_buf, sems.at[2 * N_HEAD + 1])]
            _start(small + head_copies(0), low=LEAD)
            for i in range(1, N_HEAD):
                _start(head_copies(i))
            for _, buf, sem in small:
                _wait(buf, sem)
            ffn_out = None
            for i in range(N_HEAD):
                _wait(wq_buf.at[:, :, pl.ds(i * QCOLS, QCOLS)], sems.at[i])
                _wait(ffn_buf.at[:, :, pl.ds(FFN_CUTS[i], FFN_CUTS[i + 1] - FFN_CUTS[i])], sems.at[N_HEAD + i])
                for n in range(i * LAG // N_HEAD, (i + 1) * LAG // N_HEAD):
                    _start(kv_copies(n))
                project_q(i)
                ffn_out = swiglu(i) if i == 0 else ffn_out + swiglu(i)
            x = x_buf[...].astype(F32)
            gate = jax.nn.sigmoid(jnp.sum(x * gw_buf[...].astype(F32).reshape(1, D), axis=-1, keepdims=True))
            mix_scr[0] = jnp.broadcast_to(gate, (B, D))
            mix_scr[1] = (1.0 - gate) * ffn_out

        pl.run_scoped(head, pltpu.SemaphoreType.DMA((2 * N_HEAD + 2,)))

        def step(n, state):
            _wait(kv_buf.at[n % SLOTS], ring.at[n % LAG])
            _start(kv_copies(n + LAG))
            return attend(n, state)

        state = (jnp.zeros((G, 1), F32), jnp.zeros((G, 1), F32), jnp.zeros((G, DH), F32))
        state = lax.fori_loop(0, NSTEP - LAG, step, state)
        for n in range(NSTEP - LAG, NSTEP):
            _wait(kv_buf.at[n % SLOTS], ring.at[n % LAG])
            start_wo(n + LAG - NSTEP)
            state = attend(n, state)

        attn = [attention_columns(i) for i in range(N_TAIL)]
        y = mix_scr[1]
        for i in range(N_TAIL):
            r0, r1 = WO_CUTS[i], WO_CUTS[i + 1]
            _wait(wo_buf.at[:, pl.ds(r0, r1 - r0)], ring.at[(NSTEP + i) % LAG])
            if i + LAG < N_TAIL:
                start_wo(i + LAG)
            w = wo_buf[:, r0:r1, :].reshape(SEG * (r1 - r0), D)
            y = y + mix_scr[0] * jnp.dot(attn[i], w, preferred_element_type=F32)
        o_buf[...] = y.astype(o_buf.dtype)
        out_copy.start()

    pl.run_scoped(stream, pltpu.SemaphoreType.DMA((LAG,)))
    out_copy.wait()


@jax.jit
def pallas_gated_mix__mha_block_cached__swiglu_ffn__decode_kernel(
    A_x: jax.Array,
    A_k_cache: jax.Array,
    A_v_cache: jax.Array,
    A_wq: jax.Array,
    A_wo: jax.Array,
    B_x: jax.Array,
    B_w_gate: jax.Array,
    B_w_up: jax.Array,
    B_w_down: jax.Array,
    gate_w: jax.Array,
):
    del B_x
    cache_shape = (B, 2, NGROUPS, SK, DH)
    ffn_shape = (2, F // 2, D)
    hbm = pl.BlockSpec(memory_space=pl.ANY)
    out = pl.pallas_call(
        _kernel,
        out_shape=jax.ShapeDtypeStruct((B, D), A_x.dtype),
        in_specs=[hbm] * 9,
        out_specs=hbm,
        scratch_shapes=[
            pltpu.VMEM((SLOTS, 2, 2, B, RB, DH), BF16),
            pltpu.VMEM((B, D), BF16),
            pltpu.VMEM((D,), BF16),
            pltpu.VMEM((SEG, D // SEG, H * DH), BF16),
            pltpu.VMEM((SEG, H * DH // SEG, D), BF16),
            pltpu.VMEM((3,) + ffn_shape, BF16),
            pltpu.VMEM((B * H, DH), F32),
            pltpu.VMEM((B * H, DH), F32),
            pltpu.VMEM((2, B, D), F32),
            pltpu.VMEM((B, D), A_x.dtype),
            pltpu.SemaphoreType.DMA(()),
        ],
        compiler_params=pltpu.CompilerParams(vmem_limit_bytes=64 * 1024 * 1024),
    )(
        A_x.reshape(B, D),
        A_k_cache.reshape(cache_shape),
        A_v_cache.reshape(cache_shape),
        A_wq.reshape(SEG, D // SEG, H * DH),
        A_wo.reshape(SEG, H * DH // SEG, D),
        B_w_gate.T.reshape(ffn_shape),
        B_w_up.T.reshape(ffn_shape),
        B_w_down.reshape(ffn_shape),
        gate_w,
    )
    return out.reshape(B, 1, D)
```

```python
import jax
import jax.numpy as jnp
import numpy as np
from jax import lax
import jax.experimental.pallas as pl
import jax.experimental.pallas.tpu as pltpu

B, D, H, SK, DH, F = 4, 512, 32, 4096, 128, 1376

NGROUPS = H // 2
G = 2 * B
RB = 256
NJ = SK // RB
NSTEP = NGROUPS * NJ
LAG = 4
SLOTS = LAG + 1
SEG = 4
FFN_CUTS = (0, 176, 352, 528, F // 2)
WO_CUTS = (0, 256, 512, 704, 896, 992, H * DH // SEG)
N_HEAD, N_TAIL = len(FFN_CUTS) - 1, len(WO_CUTS) - 1
QCOLS = H * DH // N_HEAD
LEAD = 32
NT = (((1,), (1,)), ((), ()))
F32, BF16 = jnp.float32, jnp.bfloat16
LOWEST = float(np.finfo(np.float32).min)


def _interleave(a, b):
    keys = [((i + 0.5) / len(a), 0, i) for i in range(len(a))]
    keys += [((i + 0.5) / len(b), 1, i) for i in range(len(b))]
    return [(a, b)[which][i] for _, which, i in sorted(keys)]


def _pair_rows(head):
    return pl.ds((head % NGROUPS) * G + (head // NGROUPS) * B, B)


def _start(copies, low=0):
    for t, (src, dst, sem) in enumerate(copies):
        pltpu.make_async_copy(src, dst, sem).start(priority=1 if t < low else t % 2)


def _wait(buf, sem):
    pltpu.make_async_copy(buf, buf, sem).wait()


def _kernel(x_hbm, k_hbm, v_hbm, wq_hbm, wo_hbm, wg_hbm, wu_hbm, wd_hbm, gw_hbm, o_hbm,
            kv_buf, x_buf, gw_buf, wq_buf, wo_buf, ffn_buf, q_scr, attn_scr, mix_scr, o_buf):
    def project_q(i):
        w = wq_buf[:, :, i * QCOLS:(i + 1) * QCOLS].reshape(D, QCOLS)
        q = jnp.dot(x_buf[...], w, preferred_element_type=F32)
        for h in range(QCOLS // DH):
            q_scr[_pair_rows(i * (QCOLS // DH) + h), :] = q[:, h * DH:(h + 1) * DH]

    def swiglu(i):
        r0, r1 = FFN_CUTS[i], FFN_CUTS[i + 1]
        wg, wu, wd = (ffn_buf[j, :, r0:r1, :].reshape(2 * (r1 - r0), D) for j in range(3))
        g = lax.dot_general(x_buf[...], wg, NT, preferred_element_type=F32)
        u = lax.dot_general(x_buf[...], wu, NT, preferred_element_type=F32)
        hidden = g * jax.nn.sigmoid(g) * u
        return jnp.dot(hidden.astype(BF16), wd, preferred_element_type=F32)

    def attend(n, state):
        slot, g0 = n % SLOTS, (n // NJ) * G
        rows = pl.ds(g0 if isinstance(n, int) else pl.multiple_of(g0, G), G)
        first = n % NJ == 0
        m = jnp.where(first, LOWEST, state[0])
        l = jnp.where(first, 0.0, state[1])
        acc = jnp.where(first, 0.0, state[2])
        q = q_scr[rows, :].astype(BF16)
        s_all = lax.dot_general(q, kv_buf[slot, 0].reshape(G * RB, DH), NT, preferred_element_type=F32)
        pair = lax.broadcasted_iota(jnp.int32, (G, RB), 0)
        s = s_all[:, :RB]
        for p in range(1, G):
            s = jnp.where(pair == p, s_all[:, p * RB:(p + 1) * RB], s)
        s = s * (DH ** -0.5)
        m_new = jnp.maximum(m, jnp.max(s, axis=-1, keepdims=True))
        alpha = jnp.exp(m - m_new)
        e = jnp.exp(s - m_new)
        l = alpha * l + jnp.sum(e, axis=-1, keepdims=True)
        e = e.astype(BF16)
        pair = lax.broadcasted_iota(jnp.int32, (G, DH), 0)
        pv = jnp.dot(e, kv_buf[slot, 1, 0, 0], preferred_element_type=F32)
        for p in range(1, G):
            pv_p = jnp.dot(e, kv_buf[slot, 1, p // B, p % B], preferred_element_type=F32)
            pv = jnp.where(pair == p, pv_p, pv)
        acc = alpha * acc + pv
        attn_scr[rows, :] = acc / l
        return m_new, l, acc

    def attention_columns(i):
        parts = []
        for s in range(SEG):
            r = WO_CUTS[i]
            while r < WO_CUTS[i + 1]:
                head, d = divmod(s * (H * DH // SEG) + r, DH)
                n = min(DH - d, WO_CUTS[i + 1] - r)
                parts.append(attn_scr[_pair_rows(head), :][:, d:d + n])
                r += n
        return jnp.concatenate(parts, axis=1).astype(BF16)

    def stream(ring):
        def kv_copies(n):
            group, r0 = n // NJ, (n % NJ) * RB
            if not isinstance(n, int):
                r0 = pl.multiple_of(r0, RB)
            return [(src.at[b, :, group, pl.ds(r0 + r, 64)], kv_buf.at[n % SLOTS, j, :, b, pl.ds(r, 64)],
                     ring.at[n % LAG])
                    for r in range(0, RB, 64) for b in (0, 2, 1, 3) for j, src in ((1, v_hbm), (0, k_hbm))]

        def start_wo(i):
            copies = [(wo_hbm.at[s, pl.ds(r, 32)], wo_buf.at[s, pl.ds(r, 32)], ring.at[(NSTEP + i) % LAG])
                      for r in range(WO_CUTS[i], WO_CUTS[i + 1], 32) for s in range(SEG)]
            _start(copies, low=len(copies) if i >= N_TAIL - 2 else 0)

        def head(sems):
            def head_copies(i):
                wq_idx = [(pl.ds(s, 2), pl.ds(r, 8), pl.ds(i * QCOLS, QCOLS))
                          for r in range(0, D // SEG, 8) for s in range(0, SEG, 2)]
                wq = [(wq_hbm.at[idx], wq_buf.at[idx], sems.at[i]) for idx in wq_idx]
                ffn = [(src.at[:, pl.ds(r, 16)], ffn_buf.at[j, :, pl.ds(r, 16)], sems.at[N_HEAD + i])
                       for r in range(FFN_CUTS[i], FFN_CUTS[i + 1], 16)
                       for j, src in enumerate((wg_hbm, wu_hbm, wd_hbm))]
                return _interleave(wq, ffn)

            small = [(x_hbm, x_buf, sems.at[2 * N_HEAD]), (gw_hbm, gw_buf, sems.at[2 * N_HEAD + 1])]
            _start(small + head_copies(0), low=LEAD)
            for i in range(1, N_HEAD):
                _start(head_copies(i))
            for _, buf, sem in small:
                _wait(buf, sem)
            ffn_out = None
            for i in range(N_HEAD):
                _wait(wq_buf.at[:, :, pl.ds(i * QCOLS, QCOLS)], sems.at[i])
                _wait(ffn_buf.at[:, :, pl.ds(FFN_CUTS[i], FFN_CUTS[i + 1] - FFN_CUTS[i])], sems.at[N_HEAD + i])
                for n in range(i * LAG // N_HEAD, (i + 1) * LAG // N_HEAD):
                    _start(kv_copies(n))
                project_q(i)
                ffn_out = swiglu(i) if i == 0 else ffn_out + swiglu(i)
            x = x_buf[...].astype(F32)
            gate = jax.nn.sigmoid(jnp.sum(x * gw_buf[...].astype(F32).reshape(1, D), axis=-1, keepdims=True))
            mix_scr[0] = jnp.broadcast_to(gate, (B, D))
            mix_scr[1] = (1.0 - gate) * ffn_out

        pl.run_scoped(head, pltpu.SemaphoreType.DMA((2 * N_HEAD + 2,)))

        def step(n, state):
            _wait(kv_buf.at[n % SLOTS], ring.at[n % LAG])
            _start(kv_copies(n + LAG))
            return attend(n, state)

        state = (jnp.zeros((G, 1), F32), jnp.zeros((G, 1), F32), jnp.zeros((G, DH), F32))
        state = lax.fori_loop(0, NSTEP - LAG, step, state)
        for n in range(NSTEP - LAG, NSTEP):
            _wait(kv_buf.at[n % SLOTS], ring.at[n % LAG])
            start_wo(n + LAG - NSTEP)
            state = attend(n, state)

        attn = [attention_columns(i) for i in range(N_TAIL)]
        y = mix_scr[1]
        for i in range(N_TAIL):
            r0, r1 = WO_CUTS[i], WO_CUTS[i + 1]
            _wait(wo_buf.at[:, pl.ds(r0, r1 - r0)], ring.at[(NSTEP + i) % LAG])
            if i + LAG < N_TAIL:
                start_wo(i + LAG)
            w = wo_buf[:, r0:r1, :].reshape(SEG * (r1 - r0), D)
            y = y + mix_scr[0] * jnp.dot(attn[i], w, preferred_element_type=F32)
        o_buf[...] = y.astype(o_buf.dtype)
        out_copy = pltpu.make_async_copy(o_buf, o_hbm, ring.at[0])
        out_copy.start()
        out_copy.wait()

    pl.run_scoped(stream, pltpu.SemaphoreType.DMA((LAG,)))


@jax.jit
def pallas_gated_mix__mha_block_cached__swiglu_ffn__decode_kernel(
    A_x: jax.Array,
    A_k_cache: jax.Array,
    A_v_cache: jax.Array,
    A_wq: jax.Array,
    A_wo: jax.Array,
    B_x: jax.Array,
    B_w_gate: jax.Array,
    B_w_up: jax.Array,
    B_w_down: jax.Array,
    gate_w: jax.Array,
):
    del B_x
    cache_shape = (B, 2, NGROUPS, SK, DH)
    ffn_shape = (2, F // 2, D)
    hbm = pl.BlockSpec(memory_space=pl.ANY)
    out = pl.pallas_call(
        _kernel,
        out_shape=jax.ShapeDtypeStruct((B, D), A_x.dtype),
        in_specs=[hbm] * 9,
        out_specs=hbm,
        scratch_shapes=[
            pltpu.VMEM((SLOTS, 2, 2, B, RB, DH), BF16),
            pltpu.VMEM((B, D), BF16),
            pltpu.VMEM((D,), BF16),
            pltpu.VMEM((SEG, D // SEG, H * DH), BF16),
            pltpu.VMEM((SEG, H * DH // SEG, D), BF16),
            pltpu.VMEM((3,) + ffn_shape, BF16),
            pltpu.VMEM((B * H, DH), F32),
            pltpu.VMEM((B * H, DH), F32),
            pltpu.VMEM((2, B, D), F32),
            pltpu.VMEM((B, D), A_x.dtype),
        ],
        compiler_params=pltpu.CompilerParams(vmem_limit_bytes=64 * 1024 * 1024),
    )(
        A_x.reshape(B, D),
        A_k_cache.reshape(cache_shape),
        A_v_cache.reshape(cache_shape),
        A_wq.reshape(SEG, D // SEG, H * DH),
        A_wo.reshape(SEG, H * DH // SEG, D),
        B_w_gate.T.reshape(ffn_shape),
        B_w_up.T.reshape(ffn_shape),
        B_w_down.reshape(ffn_shape),
        gate_w,
    )
    return out.reshape(B, 1, D)
```
